```python
import os as _os
_os.environ.setdefault('JAX_PLATFORMS', 'cpu')
import jax
import jax.numpy as jnp

def _softmax(x, axis=-1):
    return jax.nn.softmax(x, axis=axis)

def _gelu(x):
    return jax.nn.gelu(x, approximate=True)

def _silu(x):
    return jax.nn.silu(x)

def _sigmoid(x):
    return jax.nn.sigmoid(x)

def _layernorm(x, axis=-1, eps=1e-05):
    m = jnp.mean(x, axis=axis, keepdims=True)
    v = jnp.var(x, axis=axis, keepdims=True)
    return (x - m) / jnp.sqrt(v + eps)

def _scatter_add(tgt, idx, src, axis=0):
    return tgt.at[idx].add(src)

def _segment_sum(src, seg, n):
    return jax.ops.segment_sum(src, seg, n)

class _Rng:

    def __init__(self, key):
        self._k = key

    def _next(self):
        self._k, sub = jax.random.split(self._k)
        return sub

    def normal(self, shape):
        return jax.random.normal(self._next(), shape, dtype=jnp.bfloat16)

    def randint(self, lo, hi, shape):
        return jax.random.randint(self._next(), shape, lo, hi, dtype=jnp.int32)

    def uniform(self, shape, lo=0.0, hi=1.0):
        return jax.random.uniform(self._next(), shape, jnp.bfloat16, lo, hi)

    def permutation(self, n):
        return jax.random.permutation(self._next(), n)
kernel_name = 'adaLN_cond__mha_block_cached__geglu_ffn__prompt'

def setup_inputs():
    _rng = _Rng(jax.random.key(int.from_bytes(__import__("os").urandom(4), "little")))
    _w = lambda a: (lambda t: t.astype(jnp.bfloat16) if jnp.issubdtype(t.dtype, jnp.floating) else t)(jnp.asarray(a))

    def _A_setup():
        B, Sq, D = (1, 2048, 512)
        H, Sk, Dh = (32, 2048, 128)
        return {'x': _w((lambda *s: _rng.normal(s) * 0.05)(B, Sq, D)), 'k_cache': _w((lambda *s: _rng.normal(s) * 3.2)(B, H, Sk, Dh)), 'v_cache': _w((lambda *s: _rng.normal(s) * 0.4)(B, H, Sk, Dh)), 'wq': _w((lambda *s: _rng.normal(s) * 1.6)(D, H * Dh) * D ** (-0.5)), 'wo': _w((lambda *s: _rng.normal(s) * 0.4)(H * Dh, D) * (H * Dh) ** (-0.5))}
    _A_in = _A_setup()

    def _B_setup():
        B, S, D, F = (1, 2048, 512, 1792)
        return {'x': _w((lambda *s: _rng.normal(s) * 0.05)(B, S, D)), 'w_gate': _w((lambda *s: _rng.normal(s) * 0.05)(D, F)), 'w_up': _w((lambda *s: _rng.normal(s) * 0.05)(D, F)), 'w_down': _w((lambda *s: _rng.normal(s) * 0.05)(F, D))}
    _B_in = _B_setup()
    return {'A_x': _A_in['x'], 'A_k_cache': _A_in['k_cache'], 'A_v_cache': _A_in['v_cache'], 'A_wq': _A_in['wq'], 'A_wo': _A_in['wo'], 'B_x': _B_in['x'], 'B_w_gate': _B_in['w_gate'], 'B_w_up': _B_in['w_up'], 'B_w_down': _B_in['w_down'], 'c': _w((lambda *s: _rng.normal(s) * 0.05)(1, 512) * 8.0), 'w_mod': _w((lambda *s: _rng.normal(s) * 0.05)(512, 6 * 512) * 512 ** (-0.5) * 8.0)}

def reference(A_x, A_k_cache, A_v_cache, A_wq, A_wo, B_x, B_w_gate, B_w_up, B_w_down, c, w_mod):

    def _A_ref(x, k_cache, v_cache, wq, wo):
        B, Sq, D = x.shape
        H, Dh = (32, 128)
        q = (lambda x, *d: x.transpose(*d))((x @ wq).reshape(B, Sq, H, Dh), 0, 2, 1, 3)
        scores = jnp.einsum('bhqd,bhkd->bhqk', q, k_cache) * Dh ** (-0.5)
        p = _softmax(scores, axis=-1)
        o = jnp.einsum('bhqk,bhkd->bhqd', p, v_cache)
        return (lambda x, *d: x.transpose(*d))(o, 0, 2, 1, 3).reshape(B, Sq, H * Dh) @ wo

    def _B_ref(x, w_gate, w_up, w_down):
        return _gelu(x @ w_gate) * (x @ w_up) @ w_down
    x = A_x
    mod = (_silu(c) @ w_mod).reshape(c.shape[0], 6, 1, -1)
    sa, ca, ga, sb, cb, gb = (mod[:, 0].copy(), mod[:, 1].copy(), mod[:, 2].copy(), mod[:, 3].copy(), mod[:, 4].copy(), mod[:, 5].copy())
    h = _layernorm(x, axis=-1) * (1 + ca) + sa
    x = x + ga * _A_ref(h, A_k_cache, A_v_cache, A_wq, A_wo)
    h = _layernorm(x, axis=-1) * (1 + cb) + sb
    x = x + gb * _B_ref(h, B_w_gate, B_w_up, B_w_down)
    return x
```

```python
import functools
import math

import jax
import jax.numpy as jnp
import jax.experimental.pallas as pl
import jax.experimental.pallas.tpu as pltpu

_EPS = 1e-05
_LOG2E = 1.4426950408889634


def _layernorm_f32(x):
    m = jnp.mean(x, axis=-1, keepdims=True)
    d = x - m
    v = jnp.mean(d * d, axis=-1, keepdims=True)
    return d * jax.lax.rsqrt(v + _EPS)


def _kernel(x_ref, k_ref, v_ref, wq_ref, wo_ref, wg_ref, wu_ref, wd_ref, c_ref, wmod_ref,
            o_ref, h_scr, q_scr, acc_scr, mod_scr, *, n_heads, tq, tf, scale):
    hd = pl.program_id(0)
    sq, d_model = h_scr.shape

    @pl.when(hd == 0)
    def _prologue():
        c = c_ref[...].astype(jnp.float32)
        sc = c * jax.nn.sigmoid(c)
        sc8 = jnp.broadcast_to(sc, (8, sc.shape[1])).astype(jnp.bfloat16)
        mod_scr[...] = jnp.dot(sc8, wmod_ref[...], preferred_element_type=jnp.float32)
        sa = mod_scr[0:1, 0 * d_model:1 * d_model]
        ca = mod_scr[0:1, 1 * d_model:2 * d_model]
        x = x_ref[...].astype(jnp.float32)
        h = _layernorm_f32(x) * (1.0 + ca) + sa
        h_scr[...] = h.astype(jnp.bfloat16)

    q = jnp.dot(h_scr[...], wq_ref[...], preferred_element_type=jnp.float32)
    q_scr[...] = (q * scale).astype(jnp.bfloat16)

    k = k_ref[...]
    v = v_ref[...]
    wo = wo_ref[...]

    def q_block(i, carry):
        r0 = pl.multiple_of(i * tq, tq)
        qb = q_scr[pl.ds(r0, tq), :]
        s = jax.lax.dot_general(qb, k, (((1,), (1,)), ((), ())),
                                preferred_element_type=jnp.float32)
        m = jnp.max(s, axis=-1, keepdims=True)
        p = jnp.exp2(s - m)
        l = jnp.sum(p, axis=-1, keepdims=True)
        o = jnp.dot(p.astype(jnp.bfloat16), v, preferred_element_type=jnp.float32)
        o = o / l
        y = jnp.dot(o.astype(jnp.bfloat16), wo, preferred_element_type=jnp.float32)

        @pl.when(hd == 0)
        def _():
            acc_scr[pl.ds(r0, tq), :] = y

        @pl.when(hd != 0)
        def _():
            acc_scr[pl.ds(r0, tq), :] += y

        return carry

    jax.lax.fori_loop(0, sq // tq, q_block, 0)

    @pl.when(hd == n_heads - 1)
    def _epilogue():
        ga = mod_scr[0:1, 2 * d_model:3 * d_model]
        sb = mod_scr[0:1, 3 * d_model:4 * d_model]
        cb = mod_scr[0:1, 4 * d_model:5 * d_model]
        gb = mod_scr[0:1, 5 * d_model:6 * d_model]

        def f_block(i, carry):
            r0 = pl.multiple_of(i * tf, tf)
            x2 = x_ref[pl.ds(r0, tf), :].astype(jnp.float32) + ga * acc_scr[pl.ds(r0, tf), :]
            h2 = (_layernorm_f32(x2) * (1.0 + cb) + sb).astype(jnp.bfloat16)
            g = jnp.dot(h2, wg_ref[...], preferred_element_type=jnp.float32)
            u = jnp.dot(h2, wu_ref[...], preferred_element_type=jnp.float32)
            a = (jax.nn.gelu(g, approximate=True) * u).astype(jnp.bfloat16)
            f = jnp.dot(a, wd_ref[...], preferred_element_type=jnp.float32)
            o_ref[pl.ds(r0, tf), :] = (x2 + gb * f).astype(o_ref.dtype)
            return carry

        jax.lax.fori_loop(0, sq // tf, f_block, 0)


@jax.jit
def pallas_adaLN_cond__mha_block_cached__geglu_ffn__prompt_kernel(
    A_x: jax.Array,
    A_k_cache: jax.Array,
    A_v_cache: jax.Array,
    A_wq: jax.Array,
    A_wo: jax.Array,
    B_x: jax.Array,
    B_w_gate: jax.Array,
    B_w_up: jax.Array,
    B_w_down: jax.Array,
    c: jax.Array,
    w_mod: jax.Array,
):
    del B_x
    b, sq, d_model = A_x.shape
    _, n_heads, sk, d_head = A_k_cache.shape
    d_ff = B_w_gate.shape[1]
    assert b == 1

    tq = 512
    tf = 512
    scale = (d_head ** -0.5) * _LOG2E

    kernel = functools.partial(_kernel, n_heads=n_heads, tq=tq, tf=tf, scale=scale)

    const2 = lambda h: (0, 0)
    in_specs = [
        pl.BlockSpec((None, sq, d_model), lambda h: (0, 0, 0)),
        pl.BlockSpec((None, None, sk, d_head), lambda h: (0, h, 0, 0)),
        pl.BlockSpec((None, None, sk, d_head), lambda h: (0, h, 0, 0)),
        pl.BlockSpec((d_model, d_head), lambda h: (0, h)),
        pl.BlockSpec((d_head, d_model), lambda h: (h, 0)),
        pl.BlockSpec((d_model, d_ff), const2),
        pl.BlockSpec((d_model, d_ff), const2),
        pl.BlockSpec((d_ff, d_model), const2),
        pl.BlockSpec((1, d_model), const2),
        pl.BlockSpec((d_model, 6 * d_model), const2),
    ]
    out_specs = pl.BlockSpec((None, sq, d_model), lambda h: (0, 0, 0))

    return pl.pallas_call(
        kernel,
        grid=(n_heads,),
        in_specs=in_specs,
        out_specs=out_specs,
        out_shape=jax.ShapeDtypeStruct((b, sq, d_model), A_x.dtype),
        scratch_shapes=[
            pltpu.VMEM((sq, d_model), jnp.bfloat16),
            pltpu.VMEM((sq, d_head), jnp.bfloat16),
            pltpu.VMEM((sq, d_model), jnp.float32),
            pltpu.VMEM((8, 6 * d_model), jnp.float32),
        ],
        compiler_params=pltpu.CompilerParams(
            dimension_semantics=("arbitrary",),
            vmem_limit_bytes=100 * 1024 * 1024,
        ),
    )(A_x, A_k_cache, A_v_cache, A_wq, A_wo, B_w_gate, B_w_up, B_w_down, c, w_mod)
```

```python
import functools

import jax
import jax.numpy as jnp
import jax.experimental.pallas as pl
import jax.experimental.pallas.tpu as pltpu

_EPS = 1e-05
_LOG2E = 1.4426950408889634


def _layernorm_f32(x):
    m = jnp.mean(x, axis=-1, keepdims=True)
    d = x - m
    v = jnp.mean(d * d, axis=-1, keepdims=True)
    return d * jax.lax.rsqrt(v + _EPS)


def _kernel(x_ref, k_ref, v_ref, wq_ref, c_ref, wmod_ref, wmod_hbm, wo_hbm, wg_hbm, wu_hbm, wd_hbm,
            o_ref,
            h_scr, mod_scr, vt_scr, oall_scr, wo_scr, wg_scr, wu_scr, wd_scr, wmb_scr, sems,
            *, n_heads, tq, tf, scale, kc, lead, gap):
    step_id = pl.program_id(0)
    sq, d_model = h_scr.shape
    sk, d_head = k_ref.shape
    nq = sq // tq
    nt = sk // kc

    def weight_copies():
        return [
            pltpu.make_async_copy(wo_hbm, wo_scr, sems.at[0]),
            pltpu.make_async_copy(wg_hbm, wg_scr, sems.at[1]),
            pltpu.make_async_copy(wu_hbm, wu_scr, sems.at[2]),
            pltpu.make_async_copy(wd_hbm, wd_scr, sems.at[3]),
            pltpu.make_async_copy(wmod_hbm.at[:, pl.ds(2 * d_model, 4 * d_model)], wmb_scr,
                                  sems.at[4]),
        ]

    def silu_c8():
        c = c_ref[...].astype(jnp.float32)
        sc = c * jax.nn.sigmoid(c)
        return jnp.broadcast_to(sc, (8, sc.shape[1])).astype(jnp.bfloat16)

    @pl.when(step_id == 0)
    def _prologue():
        for cp in weight_copies():
            cp.start()
        mod_scr[:, 0:2 * d_model] = jnp.dot(silu_c8(), wmod_ref[...],
                                            preferred_element_type=jnp.float32)
        sa = mod_scr[0:1, 0 * d_model:1 * d_model]
        ca = mod_scr[0:1, 1 * d_model:2 * d_model]
        x = x_ref[...].astype(jnp.float32)
        h = _layernorm_f32(x) * (1.0 + ca) + sa
        h_scr[...] = h.astype(jnp.bfloat16)

    @pl.when(step_id < n_heads)
    def _attention_head():
        col0 = pl.multiple_of(step_id * d_head, d_head)
        q = jnp.dot(h_scr[...], wq_ref[...], preferred_element_type=jnp.float32)
        q_all = (q * scale).astype(jnp.bfloat16)
        vt_scr[...] = v_ref[...].T

        def make_block(i):
            r0 = i * tq
            st8 = {}

            def step(t):
                qb = q_all[r0:r0 + tq, :]
                st = jax.lax.dot_general(k_ref[t * kc:(t + 1) * kc, :], qb,
                                         (((1,), (1,)), ((), ())),
                                         preferred_element_type=jnp.float32)
                mt = jnp.max(st, axis=0, keepdims=True)
                if t == 0:
                    m_new = mt
                else:
                    m_new = jnp.maximum(st8['m'], mt)
                    alpha = jnp.exp2(st8['m'] - m_new)
                p = jnp.exp2(st - m_new)
                ls = jnp.sum(p.reshape(kc // 8, 8, tq), axis=0)
                pv = jnp.dot(vt_scr[:, t * kc:(t + 1) * kc], p.astype(jnp.bfloat16),
                             preferred_element_type=jnp.float32)
                if t == 0:
                    st8['l'], st8['acc'] = ls, pv
                else:
                    st8['l'] = st8['l'] * alpha + ls
                    st8['acc'] = st8['acc'] * alpha + pv
                st8['m'] = m_new

            def epi():
                lsum = jnp.sum(st8['l'], axis=0, keepdims=True)
                ot = st8['acc'] / lsum
                oall_scr[pl.ds(col0, d_head), r0:r0 + tq] = ot.astype(jnp.bfloat16)

            return [functools.partial(step, t) for t in range(nt)], [epi]

        blocks = [make_block(i) for i in range(nq)]
        order = []
        pending = []
        for i in range(nq):
            steps, epi = blocks[i]
            for t, s in enumerate(steps):
                order.append(s)
                if pending and t + 1 >= lead and (t + 1 - lead) % gap == 0:
                    order.append(pending.pop(0))
            order.extend(pending)
            pending = list(epi)
        order.extend(pending)
        for f in order:
            f()

    @pl.when(step_id == n_heads)
    def _wait_weights():
        for cp in weight_copies():
            cp.wait()
        mod_scr[:, 2 * d_model:6 * d_model] = jnp.dot(silu_c8(), wmb_scr[...],
                                                      preferred_element_type=jnp.float32)

    @pl.when(step_id >= n_heads)
    def _ffn_block():
        r0 = pl.multiple_of((step_id - n_heads) * tf, tf)
        ga = mod_scr[0:1, 2 * d_model:3 * d_model]
        sb = mod_scr[0:1, 3 * d_model:4 * d_model]
        cb = mod_scr[0:1, 4 * d_model:5 * d_model]
        gb = mod_scr[0:1, 5 * d_model:6 * d_model]
        attn = jax.lax.dot_general(oall_scr[:, pl.ds(r0, tf)], wo_scr[...],
                                   (((0,), (0,)), ((), ())),
                                   preferred_element_type=jnp.float32)
        x2 = x_ref[pl.ds(r0, tf), :].astype(jnp.float32) + ga * attn
        h2 = (_layernorm_f32(x2) * (1.0 + cb) + sb).astype(jnp.bfloat16)
        g = jnp.dot(h2, wg_scr[...], preferred_element_type=jnp.float32)
        u = jnp.dot(h2, wu_scr[...], preferred_element_type=jnp.float32)
        a = (jax.nn.gelu(g, approximate=True) * u).astype(jnp.bfloat16)
        f = jnp.dot(a, wd_scr[...], preferred_element_type=jnp.float32)
        o_ref[...] = (x2 + gb * f).astype(o_ref.dtype)


@jax.jit
def pallas_adaLN_cond__mha_block_cached__geglu_ffn__prompt_kernel(
    A_x: jax.Array,
    A_k_cache: jax.Array,
    A_v_cache: jax.Array,
    A_wq: jax.Array,
    A_wo: jax.Array,
    B_x: jax.Array,
    B_w_gate: jax.Array,
    B_w_up: jax.Array,
    B_w_down: jax.Array,
    c: jax.Array,
    w_mod: jax.Array,
):
    del B_x
    b, sq, d_model = A_x.shape
    _, n_heads, sk, d_head = A_k_cache.shape
    d_ff = B_w_gate.shape[1]
    assert b == 1

    tq = 256
    tf = 512
    kc = 128
    scale = (d_head ** -0.5) * _LOG2E
    n_ffn = sq // tf

    kernel = functools.partial(_kernel, n_heads=n_heads, tq=tq, tf=tf, scale=scale, kc=kc,
                               lead=5, gap=4)

    last = n_heads - 1
    head_idx = lambda s: jnp.minimum(s, last)
    const2 = lambda s: (0, 0)
    in_specs = [
        pl.BlockSpec((None, sq, d_model), lambda s: (0, 0, 0)),
        pl.BlockSpec((None, None, sk, d_head), lambda s: (0, head_idx(s), 0, 0)),
        pl.BlockSpec((None, None, sk, d_head), lambda s: (0, head_idx(s), 0, 0)),
        pl.BlockSpec((d_model, d_head), lambda s: (0, head_idx(s))),
        pl.BlockSpec((1, d_model), const2),
        pl.BlockSpec((d_model, 2 * d_model), const2),
        pl.BlockSpec(memory_space=pl.ANY),
        pl.BlockSpec(memory_space=pl.ANY),
        pl.BlockSpec(memory_space=pl.ANY),
        pl.BlockSpec(memory_space=pl.ANY),
        pl.BlockSpec(memory_space=pl.ANY),
    ]
    out_specs = pl.BlockSpec((None, tf, d_model),
                             lambda s: (0, jnp.maximum(s - n_heads, 0), 0))

    return pl.pallas_call(
        kernel,
        grid=(n_heads + n_ffn,),
        in_specs=in_specs,
        out_specs=out_specs,
        out_shape=jax.ShapeDtypeStruct((b, sq, d_model), A_x.dtype),
        scratch_shapes=[
            pltpu.VMEM((sq, d_model), jnp.bfloat16),
            pltpu.VMEM((8, 6 * d_model), jnp.float32),
            pltpu.VMEM((d_head, sk), jnp.bfloat16),
            pltpu.VMEM((n_heads * d_head, sq), jnp.bfloat16),
            pltpu.VMEM((n_heads * d_head, d_model), jnp.bfloat16),
            pltpu.VMEM((d_model, d_ff), jnp.bfloat16),
            pltpu.VMEM((d_model, d_ff), jnp.bfloat16),
            pltpu.VMEM((d_ff, d_model), jnp.bfloat16),
            pltpu.VMEM((d_model, 4 * d_model), jnp.bfloat16),
            pltpu.SemaphoreType.DMA((5,)),
        ],
        compiler_params=pltpu.CompilerParams(
            dimension_semantics=("arbitrary",),
            vmem_limit_bytes=100 * 1024 * 1024,
        ),
    )(A_x, A_k_cache, A_v_cache, A_wq, c, w_mod, w_mod, A_wo, B_w_gate, B_w_up, B_w_down)
```
